```python
import os as _os
_os.environ.setdefault("JAX_PLATFORMS", "cpu")
import jax
import jax.numpy as jnp

def _softmax(x, axis=-1):
    return jax.nn.softmax(x, axis=axis)
def _gelu(x):
    return jax.nn.gelu(x, approximate=True)
def _silu(x):
    return jax.nn.silu(x)
def _sigmoid(x):
    return jax.nn.sigmoid(x)
def _layernorm(x, axis=-1, eps=1e-5):
    m = jnp.mean(x, axis=axis, keepdims=True)
    v = jnp.var(x, axis=axis, keepdims=True)
    return (x - m) / jnp.sqrt(v + eps)
def _scatter_add(tgt, idx, src, axis=0):
    return tgt.at[idx].add(src)
def _segment_sum(src, seg, n):
    return jax.ops.segment_sum(src, seg, n)
class _Rng:
    def __init__(self, key):
        self._k = key
    def _next(self):
        self._k, sub = jax.random.split(self._k)
        return sub
    def normal(self, shape):
        return jax.random.normal(self._next(), shape, dtype=jnp.bfloat16)
    def randint(self, lo, hi, shape):
        return jax.random.randint(self._next(), shape, lo, hi, dtype=jnp.int32)
    def uniform(self, shape, lo=0.0, hi=1.0):
        return jax.random.uniform(self._next(), shape, jnp.bfloat16, lo, hi)
    def permutation(self, n):
        return jax.random.permutation(self._next(), n)


kernel_name = 'sequential_preLN__sliding_block__mixer_channel_mlp__prompt'

def setup_inputs():
    _rng = _Rng(jax.random.key(int.from_bytes(__import__("os").urandom(4), "little")))
    _w = (lambda a: (lambda t: t.astype(jnp.bfloat16) if jnp.issubdtype(t.dtype, jnp.floating) else t)(jnp.asarray(a)))
    def _A_setup():
        B, S, D = 1, 2048, 1024
        return {
            "x": _w((lambda *s: _rng.normal(s) * 0.05)(B, S, D)),
            "wqkv": _w((lambda *s: _rng.normal(s) * 0.05)(D, 3 * D)),
            "wo": _w((lambda *s: _rng.normal(s) * 0.05)(D, D)),
        }
    _A_in = _A_setup()

    def _B_setup():
        B, S, D, F = 1, 2048, 1024, 3584
        return {
            "x": _w((lambda *s: _rng.normal(s) * 0.05)(B, S, D)),
            "w1": _w((lambda *s: _rng.normal(s) * 0.8)(D, F) * (D ** -0.5)),
            "b1": _w((lambda *s: _rng.normal(s) * 0.8)(F)),
            "w2": _w((lambda *s: _rng.normal(s) * 0.8)(F, D) * (F ** -0.5)),
            "b2": _w((lambda *s: _rng.normal(s) * 0.05)(D)),
        }
    _B_in = _B_setup()

    return {
        "A_x": _A_in["x"],
        "A_wqkv": _A_in["wqkv"],
        "A_wo": _A_in["wo"],
        "B_x": _B_in["x"],
        "B_w1": _B_in["w1"],
        "B_b1": _B_in["b1"],
        "B_w2": _B_in["w2"],
        "B_b2": _B_in["b2"],
    }

def reference(A_x, A_wqkv, A_wo, B_x, B_w1, B_b1, B_w2, B_b2):
    def _A_ref(x, wqkv, wo):
        B, S, D = x.shape
        H = 32; Dh = D // H; W = 256
        qkv = (lambda x, *d: x.transpose(*d))((x @ wqkv).reshape(B, S, 3, H, Dh), 2, 0, 3, 1, 4)
        q, k, v = qkv[0], qkv[1], qkv[2]
        scores = jnp.einsum("bhqd,bhkd->bhqk", q, k) * (Dh ** -0.5)
        idx = jnp.arange(S)
        mask = (idx[:, None] - idx[None, :] >= 0) & (idx[:, None] - idx[None, :] < W)
        scores = jnp.where(mask[None, None], scores, -1e9)
        p = _softmax(scores, axis=-1)
        o = jnp.einsum("bhqk,bhkd->bhqd", p, v)
        return (lambda x, *d: x.transpose(*d))(o, 0, 2, 1, 3).reshape(B, S, D) @ wo

    def _B_ref(x, w1, b1, w2, b2):
        y = _layernorm(x, axis=-1)
        h = _gelu(jnp.einsum("bsd,df->bsf", y, w1) + b1)
        return jnp.einsum("bsf,fd->bsd", h, w2) + b2

    x = A_x
    h = x + _A_ref(_layernorm(x, axis=-1), A_wqkv, A_wo)
    h2 = h + _B_ref(_layernorm(h, axis=-1), B_w1, B_b1, B_w2, B_b2)
    return h2
```

```python
import functools

import jax
import jax.numpy as jnp
import jax.experimental.pallas as pl
import jax.experimental.pallas.tpu as pltpu

S, D, H, DH, WIN, F = 2048, 1024, 32, 32, 256, 3584
TM = 256
NB = S // TM
QB = 128
NQB = TM // QB
NG = D // 128
FC = 512
NFC = F // FC
NFUSED = 3
QC = 512
NQC = 3 * D // QC
LN_EPS = 1e-5
NEG = -1e9
QSCALE = (DH ** -0.5) * 1.4426950408889634
GELU_C = 0.7978845608028654
SCOPES = False
W4 = 4 * QB
CH = 16

f32 = jnp.float32
bf16 = jnp.bfloat16


class _Null:
    def __enter__(self):
        return self

    def __exit__(self, *a):
        return False


def _scope(name):
    return jax.named_scope(name) if SCOPES else _Null()


def _ln(v):
    m = jnp.mean(v, axis=-1, keepdims=True)
    c = v - m
    var = jnp.mean(c * c, axis=-1, keepdims=True)
    return c * jax.lax.rsqrt(var + LN_EPS)


def _gelu(y):
    u = y * (GELU_C + (GELU_C * 0.044715) * (y * y))
    hy = 0.5 * y
    return hy + hy * jnp.tanh(u)


def _dot(a, b):
    return jnp.dot(a, b, preferred_element_type=f32)


def _colmax(a):
    return jnp.max(a.reshape(a.shape[0] // 8, 8, a.shape[1]), axis=0)


def _colsum(a):
    return jnp.sum(a.reshape(a.shape[0] // 8, 8, a.shape[1]), axis=0)


def _kernel(x_ref, wqkv_hbm, wo_hbm, w1_hbm, b1_ref, w2_hbm, b2_ref, o_ref,
            wqkv_v, wo_v, w1_v, w2_v, k_scr, vt_scr, qt_scr, o_scr, xn_scr, hn_scr, acc_scr, g_scr,
            s_scr, b1_scr, b2_scr, sems):
    step = pl.program_id(0)
    cur = step % 2
    prv = 1 - cur
    kb0 = step * NQB

    def qkv_copy(c):
        return pltpu.make_async_copy(wqkv_hbm.at[:, pl.ds(c * QC, QC)],
                                     wqkv_v.at[:, pl.ds(c * QC, QC)], sems.at[c])

    def wo_copy():
        return pltpu.make_async_copy(wo_hbm, wo_v, sems.at[NQC])

    def w1_copy(c):
        return pltpu.make_async_copy(w1_hbm.at[:, pl.ds(c * FC, FC)],
                                     w1_v.at[:, pl.ds(c * FC, FC)], sems.at[NQC + 1 + c])

    def w2_copy(c):
        return pltpu.make_async_copy(w2_hbm.at[pl.ds(c * FC, FC), :],
                                     w2_v.at[pl.ds(c * FC, FC), :], sems.at[NQC + 1 + NFC + c])

    def ln1():
        xn_scr[...] = _ln(x_ref[...].astype(f32)).astype(bf16)

    def proj_k(lo=0, n=D):
        r = _dot(xn_scr[...], wqkv_v[:, D + lo:D + lo + n])
        for qb in range(NQB):
            k_scr[kb0 + qb, :, lo:lo + n] = r[qb * QB:(qb + 1) * QB].astype(bf16)

    def proj_q(lo=0, n=D):
        r = _dot(xn_scr[...], wqkv_v[:, lo:lo + n])
        for qb in range(NQB):
            for t in range(n // 128):
                blk = r[qb * QB:(qb + 1) * QB, t * 128:(t + 1) * 128] * QSCALE
                qt_scr[qb, lo + t * 128:lo + (t + 1) * 128, :] = blk.T.astype(bf16)

    def proj_v(lo=0, n=D):
        r = _dot(xn_scr[...], wqkv_v[:, 2 * D + lo:2 * D + lo + n])
        for qb in range(NQB):
            for t in range(n // 128):
                blk = r[qb * QB:(qb + 1) * QB, t * 128:(t + 1) * 128]
                vt_scr[kb0 + qb, lo + t * 128:lo + (t + 1) * 128, :] = blk.T.astype(bf16)

    def masks():
        kj = jax.lax.broadcasted_iota(jnp.int32, (QB, W4), 0)
        qi = jax.lax.broadcasted_iota(jnp.int32, (QB, W4), 1) & (QB - 1)
        causal = kj <= qi
        return causal, causal[:, 0:QB]

    def qk(u, nprev, causal):
        qb, g = divmod(u, NG)
        gb = kb0 + qb
        slot = u % 2
        lanes = slice(g * 128, (g + 1) * 128)
        k2 = k_scr[gb, :, lanes]
        parts = []
        if nprev == 2:
            k0 = k_scr[gb - 2, :, lanes]
            for c in range(QB // CH):
                parts.append(k0[c * CH:(c + 1) * CH])
                parts.append(k2[c * CH:(c + 1) * CH])
        else:
            parts.append(k2)
        if nprev >= 1:
            parts.append(k_scr[gb - 1, :, lanes])
        kwin = jnp.concatenate(parts, axis=0) if len(parts) > 1 else parts[0]
        qt = qt_scr[qb, lanes, :]
        zeros32 = jnp.zeros((DH, QB), bf16)
        cols = []
        for h in range(4):
            p4 = [zeros32] * 4
            p4[h] = qt[h * DH:(h + 1) * DH]
            cols.append(jnp.concatenate(p4, axis=0))
        wq = jnp.concatenate(cols, axis=1)
        st = _dot(kwin, wq)
        if nprev == 2:
            s02 = st[0:2 * QB].reshape(QB // CH, 2, CH, W4)
            sm = jnp.where(causal, s02[:, 1].reshape(QB, W4), s02[:, 0].reshape(QB, W4))
            rest = st[2 * QB:3 * QB]
        else:
            sm = jnp.where(causal, st[0:QB], NEG)
            rest = st[QB:2 * QB] if nprev == 1 else None
        s_scr[slot, 0:QB] = sm
        m8 = _colmax(sm)
        if rest is not None:
            s_scr[slot, QB:2 * QB] = rest
            m8 = jnp.maximum(m8, _colmax(rest))
        return jnp.max(m8, axis=0, keepdims=True)

    def softmax_pv(u, nprev, m, causal1):
        qb, g = divmod(u, NG)
        gb = kb0 + qb
        slot = u % 2
        lanes = slice(g * 128, (g + 1) * 128)
        vts = [vt_scr[gb - nprev + t, lanes, :] for t in range(nprev + 1)]
        vtwin = jnp.concatenate(vts, axis=1) if nprev else vts[0]
        nrow = QB * (2 if nprev else 1)
        outs = []
        for h in range(4):
            hl = slice(h * QB, (h + 1) * QB)
            p = jnp.exp2(s_scr[slot, 0:nrow, hl] - m[:, hl])
            l = jnp.sum(_colsum(p), axis=0, keepdims=True)
            pm = p[0:QB]
            if nprev == 2:
                pt = jnp.concatenate([jnp.where(causal1, 0.0, pm), p[QB:2 * QB],
                                      jnp.where(causal1, pm, 0.0)], axis=0)
            elif nprev == 1:
                pt = jnp.concatenate([p[QB:2 * QB], pm], axis=0)
            else:
                pt = pm
            outs.append(_dot(vtwin[h * DH:(h + 1) * DH], pt.astype(bf16)) * (1.0 / l))
        otg = jnp.concatenate(outs, axis=0)
        o_scr[qb * QB:(qb + 1) * QB, lanes] = otg.T.astype(bf16)

    def wo_proj():
        h1 = x_ref[...].astype(f32) + _dot(o_scr[...], wo_v[...])
        return h1

    def ln2(h1):
        hn_scr[cur] = _ln(h1).astype(bf16)
        acc_scr[cur] = h1 + b2_scr[...]

    def mlp_up(c, lo, n):
        if isinstance(c, int):
            off = c * FC + lo
            w = w1_v[:, off:off + n]
            b = b1_scr[:, off:off + n]
        else:
            off = pl.multiple_of(c * FC + lo, 128)
            w = w1_v[:, pl.ds(off, n)]
            b = b1_scr[:, pl.ds(off, n)]
        y = _dot(hn_scr[prv], w) + b
        g_scr[:, lo:lo + n] = _gelu(y).astype(bf16)

    def mlp_down(c, lo, n):
        if isinstance(c, int):
            w = w2_v[c * FC:(c + 1) * FC, lo:lo + n]
        else:
            w = w2_v[pl.ds(pl.multiple_of(c * FC, 128), FC), lo:lo + n]
        acc_scr[prv, :, lo:lo + n] = acc_scr[prv, :, lo:lo + n] + _dot(g_scr[...], w)

    @pl.when(step == 0)
    def _():
        with _scope("first"):
            qkv_copy(2).start()
            qkv_copy(3).start()
            qkv_copy(0).start()
            for c in range(NFC):
                b1_scr[:, c * FC:(c + 1) * FC] = b1_ref[pl.ds(c * FC, FC)].astype(f32).reshape(1, FC)
            b2_scr[...] = b2_ref[...].astype(f32).reshape(1, D)
            ln1()
            qkv_copy(2).wait()
            qkv_copy(1).start()
            proj_k(0, QC)
            qkv_copy(3).wait()
            qkv_copy(4).start()
            proj_k(QC, QC)
            qkv_copy(0).wait()
            qkv_copy(5).start()
            wo_copy().start()
            proj_q(0, QC)
            qkv_copy(1).wait()
            w1_copy(0).start()
            w2_copy(0).start()
            proj_q(QC, QC)
            qkv_copy(4).wait()
            for c in range(1, NFUSED):
                w1_copy(c).start()
                w2_copy(c).start()
            proj_v(0, QC)
            qkv_copy(5).wait()
            for c in range(NFUSED, NFC):
                w1_copy(c).start()
                w2_copy(c).start()
            proj_v(QC, QC)
            causal, causal1 = masks()
            nu = NQB * NG
            m_next = qk(0, 0, causal)
            for u in range(nu):
                m_cur = m_next
                if u + 1 < nu:
                    m_next = qk(u + 1, (u + 1) // NG, causal)
                softmax_pv(u, u // NG, m_cur, causal1)
            wo_copy().wait()
            h1 = wo_proj()
            ln2(h1)
            w1_copy(0).wait()
            w2_copy(0).wait()

    @pl.when(jnp.logical_and(step > 0, step < NB))
    def _():
        with _scope("fused"):
            pieces = []
            for c in range(NFUSED):
                pieces += [("up", c, lo) for lo in range(0, FC, 128)]
                pieces += [("down", c, lo) for lo in range(0, D, 256)]
            pieces = pieces[::-1]

            def emit(n=1):
                for _ in range(n):
                    if pieces:
                        kind, c, lo = pieces.pop()
                        if kind == "up":
                            mlp_up(c, lo, 128)
                        else:
                            mlp_down(c, lo, 256)

            emit(2)
            ln1()
            proj_k()
            proj_q()
            proj_v()

            @pl.when(step == 1)
            def _():
                for c in range(1, NFUSED):
                    w1_copy(c).wait()
                    w2_copy(c).wait()

            causal, causal1 = masks()
            nu = NQB * NG
            m_next = qk(0, 2, causal)
            for u in range(nu):
                m_cur = m_next
                if u + 1 < nu:
                    m_next = qk(u + 1, 2, causal)
                emit(1)
                softmax_pv(u, 2, m_cur, causal1)
            h1 = wo_proj()
            emit(2)
            ln2(h1)
            emit(len(pieces))

    with _scope("mlp"):
        def mlp_body(c, carry):
            @pl.when(step == 1)
            def _():
                w1_copy(c).wait()
                w2_copy(c).wait()

            mlp_up(c, 0, FC)
            mlp_down(c, 0, D)
            return carry

        lo = jnp.where(step == 0, NFC, jnp.where(step == NB, 0, NFUSED))
        jax.lax.fori_loop(lo, NFC, mlp_body, 0)

        @pl.when(step > 0)
        def _():
            o_ref[...] = acc_scr[prv].astype(o_ref.dtype)


@jax.jit
def pallas_sequential_preLN__sliding_block__mixer_channel_mlp__prompt_kernel(
    A_x: jax.Array,
    A_wqkv: jax.Array,
    A_wo: jax.Array,
    B_x: jax.Array,
    B_w1: jax.Array,
    B_b1: jax.Array,
    B_w2: jax.Array,
    B_b2: jax.Array,
):
    del B_x
    any_spec = pl.BlockSpec(memory_space=pl.ANY)
    return pl.pallas_call(
        _kernel,
        grid=(NB + 1,),
        in_specs=[
            pl.BlockSpec((None, TM, D), lambda i: (0, jnp.minimum(i, NB - 1), 0)),
            any_spec, any_spec, any_spec,
            pl.BlockSpec((F,), lambda i: (0,)),
            any_spec,
            pl.BlockSpec((D,), lambda i: (0,)),
        ],
        out_specs=pl.BlockSpec((None, TM, D), lambda i: (0, jnp.maximum(i - 1, 0), 0)),
        out_shape=jax.ShapeDtypeStruct((1, S, D), bf16),
        scratch_shapes=[
            pltpu.VMEM((D, 3 * D), bf16),
            pltpu.VMEM((D, D), bf16),
            pltpu.VMEM((D, F), bf16),
            pltpu.VMEM((F, D), bf16),
            pltpu.VMEM((S // QB, QB, D), bf16),
            pltpu.VMEM((S // QB, D, QB), bf16),
            pltpu.VMEM((NQB, D, QB), bf16),
            pltpu.VMEM((TM, D), bf16),
            pltpu.VMEM((TM, D), bf16),
            pltpu.VMEM((2, TM, D), bf16),
            pltpu.VMEM((2, TM, D), f32),
            pltpu.VMEM((TM, FC), bf16),
            pltpu.VMEM((2, 2 * QB, W4), f32),
            pltpu.VMEM((1, F), f32),
            pltpu.VMEM((1, D), f32),
            pltpu.SemaphoreType.DMA((NQC + 1 + 2 * NFC,)),
        ],
        compiler_params=pltpu.CompilerParams(
            dimension_semantics=("arbitrary",),
            vmem_limit_bytes=100 * 1024 * 1024,
        ),
        name="fused_block",
    )(A_x, A_wqkv, A_wo, B_w1, B_b1, B_w2, B_b2)
```

```python
import os as _os
import jax
import jax.numpy as jnp
import jax.experimental.pallas as pl
import jax.experimental.pallas.tpu as pltpu

S, D, H, DH, WIN, F = 2048, 1024, 32, 32, 256, 3584
TM = 256
NB = S // TM
QB = 128
HQ = QB // 2
NQB = TM // QB
NKB = S // QB
NG = D // 128
W4 = 4 * QB
FC = 512
NFC = F // FC
NLOOP = 3
UPW = int(_os.environ.get('UPW', 128))
DNW = int(_os.environ.get('DNW', 256))
EPU = [int(v) for v in _os.environ.get('EPU', '2').split(',')]
EWO = int(_os.environ.get('EWO', 2))
LNS = int(_os.environ.get('LNS', 1))
ELN = int(_os.environ.get('ELN', 0))
STU = int(_os.environ.get('STU', 0))
QC = 512
NQC = 3 * D // QC
NXB = 3
LN_EPS = 1e-5
NEG = -1e9
QSCALE = (DH ** -0.5) * 1.4426950408889634
GELU_C = 0.7978845608028654
SCOPES = False

f32 = jnp.float32
bf16 = jnp.bfloat16


class _Null:
    def __enter__(self):
        return self

    def __exit__(self, *a):
        return False


def _scope(name):
    return jax.named_scope(name) if SCOPES else _Null()


def _ds(start, size, align):
    if isinstance(start, int):
        return slice(start, start + size)
    return pl.ds(pl.multiple_of(start, align), size)


def _ln(v):
    m = jnp.mean(v, axis=-1, keepdims=True)
    c = v - m
    var = jnp.mean(c * c, axis=-1, keepdims=True)
    return c * jax.lax.rsqrt(var + LN_EPS)


def _gelu(y):
    u = y * (GELU_C + (GELU_C * 0.044715) * (y * y))
    hy = 0.5 * y
    return hy + hy * jnp.tanh(u)


def _dot(a, b):
    return jnp.dot(a, b, preferred_element_type=f32)


def _rot(a):
    return pltpu.roll(a, HQ, 1)


def _colmax(a):
    return jnp.max(a.reshape(a.shape[0] // 8, 8, a.shape[1]), axis=0)


def _colsum(a):
    return jnp.sum(a.reshape(a.shape[0] // 8, 8, a.shape[1]), axis=0)


def _kernel(x_hbm, wqkv_hbm, wo_hbm, w1_hbm, b1_hbm, w2_hbm, b2_hbm, o_ref,
            wqkv_v, wo_v, w1_v, w2_v, x_buf, k_scr, t_scr, o_scr, cs_scr, hn_scr, acc_scr,
            hn_nxt, acc_nxt, g_scr, s_scr, b1_scr, b2_scr, st_scr, b1_raw, b2_raw, sems, xsems, bsems):
    step = pl.program_id(0)
    kb0 = step * NQB

    def x_copy(b):
        return pltpu.make_async_copy(x_hbm.at[0, _ds(b * TM, TM, TM), :], x_buf.at[b % NXB],
                                     xsems.at[b % NXB])

    def qkv_copy(c):
        cols = _ds(c * QC, QC, QC)
        return pltpu.make_async_copy(wqkv_hbm.at[:, cols], wqkv_v.at[:, cols], sems.at[c])

    def wo_copy():
        return pltpu.make_async_copy(wo_hbm, wo_v, sems.at[NQC])

    def w1_copy(c):
        cols = _ds(c * FC, FC, FC)
        return pltpu.make_async_copy(w1_hbm.at[:, cols], w1_v.at[:, cols], sems.at[NQC + 1 + c])

    def w2_copy(c):
        rows = _ds(c * FC, FC, FC)
        return pltpu.make_async_copy(w2_hbm.at[rows, :], w2_v.at[rows, :], sems.at[NQC + 1 + NFC + c])

    def ln1_stats(b):
        xf = x_buf[b % NXB].astype(f32)
        m = jnp.mean(xf, axis=-1, keepdims=True)
        c = xf - m
        var = jnp.mean(c * c, axis=-1, keepdims=True)
        rstd = jax.lax.rsqrt(var + LN_EPS)
        st_scr[0] = jnp.broadcast_to(rstd, (TM, 128))
        st_scr[1] = jnp.broadcast_to(rstd * m, (TM, 128))

    def proj(col, n, first):
        cols = _ds(col, n, 128)
        lhs = x_buf[step % NXB]
        if first:
            lhs = jnp.concatenate([lhs, jnp.ones((16, D), bf16)], axis=0)
        r = _dot(lhs, wqkv_v[:, cols])
        if first:
            csum = r[TM:TM + 1]
            cs_scr[:, cols] = csum
        else:
            csum = cs_scr[:, cols]
        rstd = st_scr[0]
        shift = st_scr[1]
        return [r[0:TM, t * 128:(t + 1) * 128] * rstd - shift * csum[:, t * 128:(t + 1) * 128]
                for t in range(n // 128)]

    def store_rows(tiles, blk, lo):
        for t, r in enumerate(tiles):
            for qb in range(NQB):
                k_scr[blk + qb, :, _ds(lo + t * 128, 128, 128)] = r[qb * QB:(qb + 1) * QB].astype(bf16)

    def store_transposed(tiles, blk, lo, scale, rotate):
        for t, r in enumerate(tiles):
            for qb in range(NQB):
                b = r[qb * QB:(qb + 1) * QB]
                bt = (b if scale is None else b * scale).T
                if rotate is not None:
                    odd = [_rot(bt[h * DH:(h + 1) * DH]) for h in (1, 3)]
                    if rotate is not True:
                        odd = [jnp.where(rotate, odd[0], bt[DH:2 * DH]),
                               jnp.where(rotate, odd[1], bt[3 * DH:4 * DH])]
                    bt = jnp.concatenate([bt[0:DH], odd[0], bt[2 * DH:3 * DH], odd[1]], axis=0)
                t_scr[blk + qb, _ds(lo + t * 128, 128, 128), :] = bt.astype(bf16)

    def masks():
        kj = jax.lax.broadcasted_iota(jnp.int32, (QB, W4), 0)
        lane = jax.lax.broadcasted_iota(jnp.int32, (QB, W4), 1)
        qi = (lane + ((lane >> 7) & 1) * HQ) & (QB - 1)
        return kj <= qi

    def qk(qb, g, slot, nprev, causal):
        gb = kb0 + qb
        klanes = _ds(g * 128, 128, 128)
        k2 = k_scr[gb, :, klanes]
        qt = t_scr[NKB + qb, klanes, :]
        qh = [qt[h * DH:(h + 1) * DH] for h in range(4)]
        zeros32 = jnp.zeros((DH, QB), bf16)

        def wtile(rows):
            return jnp.concatenate([rows.get(h, zeros32) for h in range(4)], axis=0)

        wq = jnp.concatenate([wtile({h: qh[h]}) for h in range(4)], axis=1)
        if nprev == 2:
            k0 = k_scr[gb - 2, :, klanes]
            low = jax.lax.broadcasted_iota(jnp.int32, (DH, QB), 1) < HQ
            w_lo = jnp.concatenate(
                [wtile({a: jnp.where(low, qh[a], zeros32), a + 1: jnp.where(low, zeros32, qh[a + 1])})
                 for a in (0, 2)], axis=1)
            w_hi = jnp.concatenate(
                [wtile({a: jnp.where(low, zeros32, qh[a]), a + 1: jnp.where(low, qh[a + 1], zeros32)})
                 for a in (0, 2)], axis=1)
            t0 = _dot(k0[0:HQ], w_lo)
            t2 = _dot(k2[HQ:QB], w_hi)
            st = _dot(jnp.concatenate([k2[0:HQ], k0[HQ:QB], k_scr[gb - 1, :, klanes]], axis=0), wq)
            t0 = jnp.concatenate([t0[:, 0:QB], t0[:, 0:QB], t0[:, QB:], t0[:, QB:]], axis=1)
            t2 = jnp.concatenate([t2[:, 0:QB], t2[:, 0:QB], t2[:, QB:], t2[:, QB:]], axis=1)
            sm = jnp.concatenate([jnp.where(causal[0:HQ], st[0:HQ], t0),
                                  jnp.where(causal[HQ:QB], t2, st[HQ:QB])], axis=0)
            rest = st[QB:2 * QB]
        else:
            kwin = jnp.concatenate([k2, k_scr[gb - 1, :, klanes]], axis=0) if nprev else k2
            st = _dot(kwin, wq)
            sm = jnp.where(causal, st[0:QB], NEG)
            rest = st[QB:2 * QB] if nprev == 1 else None
        s_scr[slot, 0:QB] = sm
        m8 = _colmax(sm)
        if rest is not None:
            s_scr[slot, QB:2 * QB] = rest
            m8 = jnp.maximum(m8, _colmax(rest))
        return jnp.max(m8, axis=0, keepdims=True)

    def softmax_pv(qb, g, slot, nprev, m, causal):
        gb = kb0 + qb
        vrows = _ds(g * 128, 128, 128)
        vts = [t_scr[gb - nprev + t, vrows, :] for t in range(nprev + 1)]
        vtwin = jnp.concatenate(vts, axis=1) if nprev else vts[0]
        nrow = QB * (2 if nprev else 1)
        outs = []
        for h in range(4):
            hl = slice(h * QB, (h + 1) * QB)
            cz = causal[:, hl]
            p = jnp.exp2(s_scr[slot, 0:nrow, hl] - m[:, hl])
            l = jnp.sum(_colsum(p), axis=0, keepdims=True)
            pm = p[0:QB]
            if nprev == 2:
                pt = jnp.concatenate([jnp.where(cz, 0.0, pm), p[QB:2 * QB],
                                      jnp.where(cz, pm, 0.0)], axis=0)
            elif nprev == 1:
                pt = jnp.concatenate([p[QB:2 * QB], pm], axis=0)
            else:
                pt = pm
            o = _dot(vtwin[h * DH:(h + 1) * DH], pt.astype(bf16)) * (1.0 / l)
            outs.append(_rot(o) if h % 2 else o)
        otg = jnp.concatenate(outs, axis=0)
        o_scr[qb * QB:(qb + 1) * QB, _ds(g * 128, 128, 128)] = otg.T.astype(bf16)

    def wo_proj():
        return x_buf[step % NXB].astype(f32) + _dot(o_scr[...], wo_v[...])

    def ln2(h1, r0=0, n=TM):
        h = h1[r0:r0 + n]
        hn_nxt[r0:r0 + n] = _ln(h).astype(bf16)
        acc_nxt[r0:r0 + n] = h + b2_scr[...]

    def mlp_up(c, lo, n, hn_ref):
        cols = _ds(c * FC + lo, n, 128)
        y = _dot(hn_ref[...], w1_v[:, cols]) + b1_scr[:, cols]
        g_scr[:, lo:lo + n] = _gelu(y).astype(bf16)

    def mlp_down(c, lo, n, write_out=False, init=None):
        acc = acc_scr[:, lo:lo + n]
        if init is not None:
            acc = jnp.where(init, acc_nxt[:, lo:lo + n], acc)
        new = acc + _dot(g_scr[...], w2_v[_ds(c * FC, FC, 128), lo:lo + n])
        acc_scr[:, lo:lo + n] = new
        if write_out:
            o_ref[:, lo:lo + n] = new.astype(o_ref.dtype)

    @pl.when(jnp.logical_and(step >= 1, step + 1 < NB))
    def _():
        x_copy(step + 1).wait()

    @pl.when(jnp.logical_and(step >= 1, step + 2 < NB))
    def _():
        x_copy(step + 2).start()

    @pl.when(step == 0)
    def _():
        with _scope("first"):
            b1_copy = pltpu.make_async_copy(b1_hbm, b1_raw, bsems.at[0])
            b2_copy = pltpu.make_async_copy(b2_hbm, b2_raw, bsems.at[1])
            x_copy(0).start()
            qkv_copy(2).start()
            b1_copy.start()
            b2_copy.start()
            acc_scr[...] = jnp.zeros((TM, D), f32)
            x_copy(0).wait()
            qkv_copy(3).start()
            ln1_stats(0)
            b1_copy.wait()
            b2_copy.wait()
            for c in range(NFC):
                b1_scr[:, c * FC:(c + 1) * FC] = b1_raw[pl.ds(c * FC, FC)].astype(f32).reshape(1, FC)
            b2_scr[...] = b2_raw[...].astype(f32).reshape(1, D)
            qkv_copy(2).wait()
            qkv_copy(0).start()
            store_rows(proj(D, QC, True), 0, 0)
            qkv_copy(3).wait()
            qkv_copy(4).start()
            store_rows(proj(D + QC, QC, True), 0, QC)
            qkv_copy(0).wait()
            qkv_copy(1).start()
            store_transposed(proj(0, QC, True), NKB, 0, QSCALE, True)
            qkv_copy(4).wait()
            qkv_copy(5).start()
            x_copy(1).start()
            wo_copy().start()
            store_transposed(proj(2 * D, QC, True), 0, 0, None, None)
            causal = masks()

            def attend(groups):
                units = [(qb, g) for g in groups for qb in range(NQB)]
                m_next = qk(*units[0], 0, units[0][0], causal)
                for u in range(len(units)):
                    m_cur = m_next
                    if u + 1 < len(units):
                        m_next = qk(*units[u + 1], (u + 1) % 2, units[u + 1][0], causal)
                    softmax_pv(*units[u], u % 2, units[u][0], m_cur, causal)

            qkv_copy(1).wait()
            w1_copy(0).start()
            w2_copy(0).start()
            x_copy(2).start()
            store_transposed(proj(QC, QC, True), NKB, QC, QSCALE, True)
            attend(range(0, NG // 2))
            qkv_copy(5).wait()
            for c in range(1, NFC):
                w1_copy(c).start()
                w2_copy(c).start()
            x_copy(1).wait()
            store_transposed(proj(2 * D + QC, QC, True), 0, QC, None, None)
            attend(range(NG // 2, NG))
            ln1_stats(1)
            wo_copy().wait()
            h1 = wo_proj()
            ln2(h1)

    @pl.when(jnp.logical_and(step > 0, step < NB))
    def _():
        with _scope("proj"):
            def proj_body(j, carry):
                @pl.when(step == 1)
                def _():
                    w1_copy(j).wait()
                    w2_copy(j).wait()

                is_k, is_q, is_v = j == 0, j == 1, j == 2
                col = jnp.where(is_k, D, jnp.where(is_q, 0, 2 * D))
                mlp_up(j, 0, FC, hn_nxt)
                r = proj(col, D, False)
                store_rows(r, jnp.where(is_k, kb0, NKB), 0)
                store_transposed(r, jnp.where(is_v, kb0, jnp.where(is_q, NKB, NKB + NQB)), 0,
                                 jnp.where(is_q, QSCALE, 1.0).astype(f32), is_q)
                mlp_down(j, 0, D, init=is_k)
                hn_scr[...] = hn_nxt[...]
                return carry

            jax.lax.fori_loop(0, NLOOP, proj_body, 0)

        @pl.when(step == 1)
        def _():
            for c in range(NLOOP, NFC):
                w1_copy(c).wait()
                w2_copy(c).wait()

        with _scope("fused"):
            pieces = []
            for c in range(NLOOP, NFC):
                pieces += [("up", c, lo) for lo in range(0, FC, UPW)]
                pieces += [("down", c, lo) for lo in range(0, D, DNW)]
            pieces = pieces[::-1]

            def emit(n=1):
                for _ in range(n):
                    if pieces:
                        kind, c, lo = pieces.pop()
                        if kind == "up":
                            mlp_up(c, lo, UPW, hn_scr)
                        else:
                            mlp_down(c, lo, DNW, write_out=(c == NFC - 1))

            causal = masks()
            nu = NQB * NG
            units = [divmod(u, NG) for u in range(nu)]
            m_next = qk(*units[0], 0, 2, causal)
            for u in range(nu):
                m_cur = m_next
                if u + 1 < nu:
                    m_next = qk(*units[u + 1], (u + 1) % 2, 2, causal)
                emit(EPU[u % len(EPU)])
                softmax_pv(*units[u], u % 2, 2, m_cur, causal)
                if u == STU:
                    ln1_stats(step + 1)
            h1 = wo_proj()
            emit(EWO)
            for r0 in range(0, TM, TM // LNS):
                ln2(h1, r0, TM // LNS)
                emit(ELN)
            emit(len(pieces))

    @pl.when(step == NB)
    def _():
        with _scope("last"):
            def mlp_body(c, carry):
                mlp_up(c, 0, FC, hn_nxt)
                mlp_down(c, 0, D, write_out=True, init=(c == 0))
                return carry

            jax.lax.fori_loop(0, NFC, mlp_body, 0)


@jax.jit
def pallas_sequential_preLN__sliding_block__mixer_channel_mlp__prompt_kernel(
    A_x: jax.Array,
    A_wqkv: jax.Array,
    A_wo: jax.Array,
    B_x: jax.Array,
    B_w1: jax.Array,
    B_b1: jax.Array,
    B_w2: jax.Array,
    B_b2: jax.Array,
):
    del B_x
    any_spec = pl.BlockSpec(memory_space=pl.ANY)
    return pl.pallas_call(
        _kernel,
        grid=(NB + 1,),
        in_specs=[
            any_spec, any_spec, any_spec, any_spec, any_spec, any_spec, any_spec,
        ],
        out_specs=pl.BlockSpec((None, TM, D), lambda i: (0, jnp.maximum(i - 1, 0), 0)),
        out_shape=jax.ShapeDtypeStruct((1, S, D), bf16),
        scratch_shapes=[
            pltpu.VMEM((D, 3 * D), bf16),
            pltpu.VMEM((D, D), bf16),
            pltpu.VMEM((D, F), bf16),
            pltpu.VMEM((F, D), bf16),
            pltpu.VMEM((NXB, TM, D), bf16),
            pltpu.VMEM((NKB + NQB, QB, D), bf16),
            pltpu.VMEM((NKB + 2 * NQB, D, QB), bf16),
            pltpu.VMEM((TM, D), bf16),
            pltpu.VMEM((1, 3 * D), f32),
            pltpu.VMEM((TM, D), bf16),
            pltpu.VMEM((TM, D), f32),
            pltpu.VMEM((TM, D), bf16),
            pltpu.VMEM((TM, D), f32),
            pltpu.VMEM((TM, FC), bf16),
            pltpu.VMEM((2, 2 * QB, W4), f32),
            pltpu.VMEM((1, F), f32),
            pltpu.VMEM((1, D), f32),
            pltpu.VMEM((2, TM, 128), f32),
            pltpu.VMEM((F,), bf16),
            pltpu.VMEM((D,), bf16),
            pltpu.SemaphoreType.DMA((NQC + 1 + 2 * NFC,)),
            pltpu.SemaphoreType.DMA((NXB,)),
            pltpu.SemaphoreType.DMA((2,)),
        ],
        compiler_params=pltpu.CompilerParams(
            dimension_semantics=("arbitrary",),
            vmem_limit_bytes=100 * 1024 * 1024,
        ),
        name="fused_block",
    )(A_x, A_wqkv, A_wo, B_w1, B_b1, B_w2, B_b2)
```

```python
import jax
import jax.numpy as jnp
import jax.experimental.pallas as pl
import jax.experimental.pallas.tpu as pltpu

S, D, H, DH, WIN, F = 2048, 1024, 32, 32, 256, 3584
TM = 256
NB = S // TM
QB = 128
HQ = QB // 2
NQB = TM // QB
NKB = S // QB
NG = D // 128
W4 = 4 * QB
FC = 512
NFC = F // FC
NLOOP = 3
UPW = 128
DNW = 256
EPU = (2, 2, 1)
EWO = 2
QC = 512
NQC = 3 * D // QC
NXB = 3
SROWS = 96
FCL = 896
LN_EPS = 1e-5
NEG = -1e9
QSCALE = (DH ** -0.5) * 1.4426950408889634
GELU_C = 0.7978845608028654

f32 = jnp.float32
bf16 = jnp.bfloat16


def _ds(start, size, align):
    if isinstance(start, int):
        return slice(start, start + size)
    return pl.ds(pl.multiple_of(start, align), size)


def _ln(v):
    m = jnp.mean(v, axis=-1, keepdims=True)
    c = v - m
    var = jnp.mean(c * c, axis=-1, keepdims=True)
    return c * jax.lax.rsqrt(var + LN_EPS)


def _gelu(y):
    u = y * (GELU_C + (GELU_C * 0.044715) * (y * y))
    hy = 0.5 * y
    return hy + hy * jnp.tanh(u)


def _dot(a, b):
    return jnp.dot(a, b, preferred_element_type=f32)


def _rot(a):
    return pltpu.roll(a, HQ, 1)


def _colmax(a):
    return jnp.max(a.reshape(a.shape[0] // 8, 8, a.shape[1]), axis=0)


def _colsum(a):
    return jnp.sum(a.reshape(a.shape[0] // 8, 8, a.shape[1]), axis=0)


def _kernel(x_hbm, wqkv_hbm, wo_hbm, w1_hbm, b1_hbm, w2_hbm, b2_hbm, o_ref,
            wqkv_v, wo_v, w1_v, w2_v, x_buf, k_scr, t_scr, o_scr, cs_scr, hn_scr, acc_scr,
            hn_nxt, acc_nxt, g_scr, s_scr, b1_scr, b2_scr, st_scr, st_nxt, b1_raw, b2_raw, sems, xsems, bsems):
    step = pl.program_id(0)
    kb0 = step * NQB

    def x_copy(b):
        return pltpu.make_async_copy(x_hbm.at[0, _ds(b * TM, TM, TM), :], x_buf.at[b % NXB],
                                     xsems.at[b % NXB])

    def qkv_copy(c):
        cols = _ds(c * QC, QC, QC)
        return pltpu.make_async_copy(wqkv_hbm.at[:, cols], wqkv_v.at[:, cols], sems.at[c])

    def wo_copy():
        return pltpu.make_async_copy(wo_hbm, wo_v, sems.at[NQC])

    def w1_copy(c):
        cols = _ds(c * FC, FC, FC)
        return pltpu.make_async_copy(w1_hbm.at[:, cols], w1_v.at[:, cols], sems.at[NQC + 1 + c])

    def w2_copy(c):
        rows = _ds(c * FC, FC, FC)
        return pltpu.make_async_copy(w2_hbm.at[rows, :], w2_v.at[rows, :], sems.at[NQC + 1 + NFC + c])

    def ln1_stats(b, dst, r0=0, n=TM):
        rows = _ds(r0, n, 8)
        xf = x_buf[b % NXB, rows].astype(f32)
        m = jnp.mean(xf, axis=-1, keepdims=True)
        c = xf - m
        var = jnp.mean(c * c, axis=-1, keepdims=True)
        rstd = jax.lax.rsqrt(var + LN_EPS)
        dst[0, rows] = jnp.broadcast_to(rstd, (n, 128))
        dst[1, rows] = jnp.broadcast_to(rstd * m, (n, 128))

    def proj(col, n, first):
        cols = _ds(col, n, 128)
        lhs = x_buf[step % NXB]
        if first:
            lhs = jnp.concatenate([lhs, jnp.ones((16, D), bf16)], axis=0)
        r = _dot(lhs, wqkv_v[:, cols])
        if first:
            csum = r[TM:TM + 1]
            cs_scr[:, cols] = csum
        else:
            csum = cs_scr[:, cols]
        rstd = st_scr[0]
        shift = st_scr[1]
        return [r[0:TM, t * 128:(t + 1) * 128] * rstd - shift * csum[:, t * 128:(t + 1) * 128]
                for t in range(n // 128)]

    def store_rows(tiles, blk, lo):
        for t, r in enumerate(tiles):
            for qb in range(NQB):
                k_scr[blk + qb, :, _ds(lo + t * 128, 128, 128)] = r[qb * QB:(qb + 1) * QB].astype(bf16)

    def store_transposed(tiles, blk, lo, scale, rotate):
        for t, r in enumerate(tiles):
            for qb in range(NQB):
                b = r[qb * QB:(qb + 1) * QB]
                bt = (b if scale is None else b * scale).T
                if rotate is not None:
                    odd = [_rot(bt[h * DH:(h + 1) * DH]) for h in (1, 3)]
                    if rotate is not True:
                        odd = [jnp.where(rotate, odd[0], bt[DH:2 * DH]),
                               jnp.where(rotate, odd[1], bt[3 * DH:4 * DH])]
                    bt = jnp.concatenate([bt[0:DH], odd[0], bt[2 * DH:3 * DH], odd[1]], axis=0)
                t_scr[blk + qb, _ds(lo + t * 128, 128, 128), :] = bt.astype(bf16)

    def masks():
        kj = jax.lax.broadcasted_iota(jnp.int32, (QB, W4), 0)
        lane = jax.lax.broadcasted_iota(jnp.int32, (QB, W4), 1)
        qi = (lane + ((lane >> 7) & 1) * HQ) & (QB - 1)
        return kj <= qi

    def qk(qb, g, slot, nprev, causal):
        gb = kb0 + qb
        klanes = _ds(g * 128, 128, 128)
        k2 = k_scr[gb, :, klanes]
        qt = t_scr[NKB + qb, klanes, :]
        qh = [qt[h * DH:(h + 1) * DH] for h in range(4)]
        zeros32 = jnp.zeros((DH, QB), bf16)

        def wtile(rows):
            return jnp.concatenate([rows.get(h, zeros32) for h in range(4)], axis=0)

        wq = jnp.concatenate([wtile({h: qh[h]}) for h in range(4)], axis=1)
        if nprev == 2:
            k0 = k_scr[gb - 2, :, klanes]
            low = jax.lax.broadcasted_iota(jnp.int32, (DH, QB), 1) < HQ
            w_lo = jnp.concatenate(
                [wtile({a: jnp.where(low, qh[a], zeros32), a + 1: jnp.where(low, zeros32, qh[a + 1])})
                 for a in (0, 2)], axis=1)
            w_hi = jnp.concatenate(
                [wtile({a: jnp.where(low, zeros32, qh[a]), a + 1: jnp.where(low, qh[a + 1], zeros32)})
                 for a in (0, 2)], axis=1)
            t0 = _dot(k0[0:HQ], w_lo)
            t2 = _dot(k2[HQ:QB], w_hi)
            st = _dot(jnp.concatenate([k2[0:HQ], k0[HQ:QB], k_scr[gb - 1, :, klanes]], axis=0), wq)
            t0 = jnp.concatenate([t0[:, 0:QB], t0[:, 0:QB], t0[:, QB:], t0[:, QB:]], axis=1)
            t2 = jnp.concatenate([t2[:, 0:QB], t2[:, 0:QB], t2[:, QB:], t2[:, QB:]], axis=1)
            sm = jnp.concatenate([jnp.where(causal[0:HQ], st[0:HQ], t0),
                                  jnp.where(causal[HQ:QB], t2, st[HQ:QB])], axis=0)
            rest = st[QB:2 * QB]
        else:
            kwin = jnp.concatenate([k2, k_scr[gb - 1, :, klanes]], axis=0) if nprev else k2
            st = _dot(kwin, wq)
            sm = jnp.where(causal, st[0:QB], NEG)
            rest = st[QB:2 * QB] if nprev == 1 else None
        s_scr[slot, 0:QB] = sm
        m8 = _colmax(sm)
        if rest is not None:
            s_scr[slot, QB:2 * QB] = rest
            m8 = jnp.maximum(m8, _colmax(rest))
        return jnp.max(m8, axis=0, keepdims=True)

    def softmax_pv(qb, g, slot, nprev, m, causal):
        gb = kb0 + qb
        vrows = _ds(g * 128, 128, 128)
        vts = [t_scr[gb - nprev + t, vrows, :] for t in range(nprev + 1)]
        vtwin = jnp.concatenate(vts, axis=1) if nprev else vts[0]
        nrow = QB * (2 if nprev else 1)
        outs = []
        for h in range(4):
            hl = slice(h * QB, (h + 1) * QB)
            cz = causal[:, hl]
            p = jnp.exp2(s_scr[slot, 0:nrow, hl] - m[:, hl])
            l = jnp.sum(_colsum(p), axis=0, keepdims=True)
            pm = p[0:QB]
            if nprev == 2:
                pt = jnp.concatenate([jnp.where(cz, 0.0, pm), p[QB:2 * QB],
                                      jnp.where(cz, pm, 0.0)], axis=0)
            elif nprev == 1:
                pt = jnp.concatenate([p[QB:2 * QB], pm], axis=0)
            else:
                pt = pm
            o = _dot(vtwin[h * DH:(h + 1) * DH], pt.astype(bf16)) * (1.0 / l)
            outs.append(_rot(o) if h % 2 else o)
        otg = jnp.concatenate(outs, axis=0)
        o_scr[qb * QB:(qb + 1) * QB, _ds(g * 128, 128, 128)] = otg.T.astype(bf16)

    def wo_proj():
        return x_buf[step % NXB].astype(f32) + _dot(o_scr[...], wo_v[...])

    def ln2(h1):
        hn_nxt[...] = _ln(h1).astype(bf16)
        acc_nxt[...] = h1 + b2_scr[...]

    def mlp_up(c, lo, n, hn_ref, fc=FC):
        cols = _ds(c * fc + lo, n, 128)
        y = _dot(hn_ref[...], w1_v[:, cols]) + b1_scr[:, cols]
        g_scr[:, lo:lo + n] = _gelu(y).astype(bf16)

    def mlp_down(c, lo, n, write_out=False, init=None, fc=FC):
        acc = acc_scr[:, lo:lo + n]
        if init is not None:
            acc = jnp.where(init, acc_nxt[:, lo:lo + n], acc)
        new = acc + _dot(g_scr[:, 0:fc], w2_v[_ds(c * fc, fc, 128), lo:lo + n])
        acc_scr[:, lo:lo + n] = new
        if write_out:
            o_ref[:, lo:lo + n] = new.astype(o_ref.dtype)

    @pl.when(jnp.logical_and(step >= 1, step + 1 < NB))
    def _():
        x_copy(step + 1).wait()

    @pl.when(jnp.logical_and(step >= 1, step + 2 < NB))
    def _():
        x_copy(step + 2).start()

    @pl.when(step == 0)
    def _():
        b1_copy = pltpu.make_async_copy(b1_hbm, b1_raw, bsems.at[0])
        b2_copy = pltpu.make_async_copy(b2_hbm, b2_raw, bsems.at[1])
        x_copy(0).start()
        qkv_copy(2).start()
        b1_copy.start()
        b2_copy.start()
        acc_scr[...] = jnp.zeros((TM, D), f32)
        x_copy(0).wait()
        qkv_copy(3).start()
        ln1_stats(0, st_scr)
        b1_copy.wait()
        b2_copy.wait()
        for c in range(NFC):
            b1_scr[:, c * FC:(c + 1) * FC] = b1_raw[pl.ds(c * FC, FC)].astype(f32).reshape(1, FC)
        b2_scr[...] = b2_raw[...].astype(f32).reshape(1, D)
        qkv_copy(2).wait()
        qkv_copy(0).start()
        store_rows(proj(D, QC, True), 0, 0)
        qkv_copy(3).wait()
        qkv_copy(4).start()
        store_rows(proj(D + QC, QC, True), 0, QC)
        qkv_copy(0).wait()
        qkv_copy(1).start()
        store_transposed(proj(0, QC, True), NKB, 0, QSCALE, True)
        qkv_copy(4).wait()
        qkv_copy(5).start()
        x_copy(1).start()
        wo_copy().start()
        store_transposed(proj(2 * D, QC, True), 0, 0, None, None)
        causal = masks()

        def attend(groups):
            units = [(qb, g) for g in groups for qb in range(NQB)]
            m_next = qk(*units[0], 0, units[0][0], causal)
            for u in range(len(units)):
                m_cur = m_next
                if u + 1 < len(units):
                    m_next = qk(*units[u + 1], (u + 1) % 2, units[u + 1][0], causal)
                softmax_pv(*units[u], u % 2, units[u][0], m_cur, causal)

        qkv_copy(1).wait()
        w1_copy(0).start()
        w2_copy(0).start()
        x_copy(2).start()
        store_transposed(proj(QC, QC, True), NKB, QC, QSCALE, True)
        attend(range(0, NG // 2))
        qkv_copy(5).wait()
        for c in range(1, NFC):
            w1_copy(c).start()
            w2_copy(c).start()
        x_copy(1).wait()
        store_transposed(proj(2 * D + QC, QC, True), 0, QC, None, None)
        attend(range(NG // 2, NG))
        ln1_stats(1, st_scr)
        wo_copy().wait()
        h1 = wo_proj()
        ln2(h1)

    @pl.when(jnp.logical_and(step > 0, step < NB))
    def _():
        def proj_body(j, carry):
            @pl.when(step == 1)
            def _():
                w1_copy(j).wait()
                w2_copy(j).wait()

            is_k, is_q, is_v = j == 0, j == 1, j == 2
            col = jnp.where(is_k, D, jnp.where(is_q, 0, 2 * D))
            mlp_up(j, 0, FC, hn_nxt)
            r = proj(col, D, False)
            store_rows(r, jnp.where(is_k, kb0, NKB), 0)
            store_transposed(r, jnp.where(is_v, kb0, jnp.where(is_q, NKB, NKB + NQB)), 0,
                             jnp.where(is_q, QSCALE, 1.0).astype(f32), is_q)
            mlp_down(j, 0, D, init=is_k)
            hn_scr[...] = hn_nxt[...]
            ln1_stats(step + 1, st_nxt, jnp.minimum(j * SROWS, TM - SROWS), SROWS)
            return carry

        jax.lax.fori_loop(0, NLOOP, proj_body, 0)

        @pl.when(step == 1)
        def _():
            for c in range(NLOOP, NFC):
                w1_copy(c).wait()
                w2_copy(c).wait()

        pieces = []
        for c in range(NLOOP, NFC):
            pieces += [("up", c, lo) for lo in range(0, FC, UPW)]
            pieces += [("down", c, lo) for lo in range(0, D, DNW)]
        pieces = pieces[::-1]

        def emit(n=1):
            for _ in range(n):
                if pieces:
                    kind, c, lo = pieces.pop()
                    if kind == "up":
                        mlp_up(c, lo, UPW, hn_scr)
                    else:
                        mlp_down(c, lo, DNW, write_out=(c == NFC - 1))

        causal = masks()
        nu = NQB * NG
        units = [divmod(u, NG) for u in range(nu)]
        m_next = qk(*units[0], 0, 2, causal)
        for u in range(nu):
            m_cur = m_next
            if u + 1 < nu:
                m_next = qk(*units[u + 1], (u + 1) % 2, 2, causal)
            emit(EPU[u % len(EPU)])
            softmax_pv(*units[u], u % 2, 2, m_cur, causal)
            if u == 0:
                st_scr[...] = st_nxt[...]
        h1 = wo_proj()
        emit(EWO)
        ln2(h1)
        emit(len(pieces))

    @pl.when(step == NB)
    def _():
        def mlp_body(c, carry):
            mlp_up(c, 0, FCL, hn_nxt, FCL)
            mlp_down(c, 0, D, write_out=True, init=(c == 0), fc=FCL)
            return carry

        jax.lax.fori_loop(0, F // FCL, mlp_body, 0)


@jax.jit
def pallas_sequential_preLN__sliding_block__mixer_channel_mlp__prompt_kernel(
    A_x: jax.Array,
    A_wqkv: jax.Array,
    A_wo: jax.Array,
    B_x: jax.Array,
    B_w1: jax.Array,
    B_b1: jax.Array,
    B_w2: jax.Array,
    B_b2: jax.Array,
):
    del B_x
    any_spec = pl.BlockSpec(memory_space=pl.ANY)
    return pl.pallas_call(
        _kernel,
        grid=(NB + 1,),
        in_specs=[
            any_spec, any_spec, any_spec, any_spec, any_spec, any_spec, any_spec,
        ],
        out_specs=pl.BlockSpec((None, TM, D), lambda i: (0, jnp.maximum(i - 1, 0), 0)),
        out_shape=jax.ShapeDtypeStruct((1, S, D), bf16),
        scratch_shapes=[
            pltpu.VMEM((D, 3 * D), bf16),
            pltpu.VMEM((D, D), bf16),
            pltpu.VMEM((D, F), bf16),
            pltpu.VMEM((F, D), bf16),
            pltpu.VMEM((NXB, TM, D), bf16),
            pltpu.VMEM((NKB + NQB, QB, D), bf16),
            pltpu.VMEM((NKB + 2 * NQB, D, QB), bf16),
            pltpu.VMEM((TM, D), bf16),
            pltpu.VMEM((1, 3 * D), f32),
            pltpu.VMEM((TM, D), bf16),
            pltpu.VMEM((TM, D), f32),
            pltpu.VMEM((TM, D), bf16),
            pltpu.VMEM((TM, D), f32),
            pltpu.VMEM((TM, max(FC, FCL)), bf16),
            pltpu.VMEM((2, 2 * QB, W4), f32),
            pltpu.VMEM((1, F), f32),
            pltpu.VMEM((1, D), f32),
            pltpu.VMEM((2, TM, 128), f32),
            pltpu.VMEM((2, TM, 128), f32),
            pltpu.VMEM((F,), bf16),
            pltpu.VMEM((D,), bf16),
            pltpu.SemaphoreType.DMA((NQC + 1 + 2 * NFC,)),
            pltpu.SemaphoreType.DMA((NXB,)),
            pltpu.SemaphoreType.DMA((2,)),
        ],
        compiler_params=pltpu.CompilerParams(
            dimension_semantics=("arbitrary",),
            vmem_limit_bytes=100 * 1024 * 1024,
        ),
        name="fused_block",
    )(A_x, A_wqkv, A_wo, B_w1, B_b1, B_w2, B_b2)
```
